```python
import jax
import jax.numpy as jnp

def _softmax(x, axis=-1):
    return jax.nn.softmax(x, axis=axis)
def _gelu(x):
    return jax.nn.gelu(x, approximate=True)
def _silu(x):
    return jax.nn.silu(x)
def _sigmoid(x):
    return jax.nn.sigmoid(x)
def _layernorm(x, axis=-1, eps=1e-5):
    m = jnp.mean(x, axis=axis, keepdims=True)
    v = jnp.var(x, axis=axis, keepdims=True)
    return (x - m) / jnp.sqrt(v + eps)
def _scatter_add(tgt, idx, src, axis=0):
    return tgt.at[idx].add(src)
def _segment_sum(src, seg, n):
    return jax.ops.segment_sum(src, seg, n)
class _Rng:
    def __init__(self, key):
        self._k = key
    def _next(self):
        self._k, sub = jax.random.split(self._k)
        return sub
    def normal(self, shape):
        return jax.random.normal(self._next(), shape, dtype=jnp.bfloat16)
    def randint(self, lo, hi, shape):
        return jax.random.randint(self._next(), shape, lo, hi, dtype=jnp.int32)
    def uniform(self, shape, lo=0.0, hi=1.0):
        return jax.random.uniform(self._next(), shape, jnp.bfloat16, lo, hi)
    def permutation(self, n):
        return jax.random.permutation(self._next(), n)


kernel_name = 'interleave_layers__sliding_block__sliding_local_dilated__prompt'

def setup_inputs():
    _rng = _Rng(jax.random.key(int.from_bytes(__import__("os").urandom(4), "little")))
    _w = (lambda a: (lambda t: t.astype(jnp.bfloat16) if jnp.issubdtype(t.dtype, jnp.floating) else t)(jnp.asarray(a)))
    def _A_setup():
        B, S, D = 1, 2048, 1024
        return {
            "x": _w((lambda *s: _rng.normal(s) * 0.05)(B, S, D)),
            "wqkv": _w((lambda *s: _rng.normal(s) * 0.05)(D, 3 * D)),
            "wo": _w((lambda *s: _rng.normal(s) * 0.05)(D, D)),
        }
    _A_in = _A_setup()

    def _B_setup():
        B, S, D = 1, 2048, 1024
        return {
            "x": _w((lambda *s: _rng.normal(s) * 0.05)(B, S, D)),
            "wqkv": _w((lambda *s: _rng.normal(s) * 0.05)(D, 3 * D)),
            "wo": _w((lambda *s: _rng.normal(s) * 0.05)(D, D)),
        }
    _B_in = _B_setup()

    return {
        "A_x": _A_in["x"],
        "A_wqkv": _A_in["wqkv"],
        "A_wo": _A_in["wo"],
        "B_x": _B_in["x"],
        "B_wqkv": _B_in["wqkv"],
        "B_wo": _B_in["wo"],
    }

def reference(A_x, A_wqkv, A_wo, B_x, B_wqkv, B_wo):
    def _A_ref(x, wqkv, wo):
        B, S, D = x.shape
        H = 32; Dh = D // H; W = 256
        qkv = (lambda x, *d: x.transpose(*d))((x @ wqkv).reshape(B, S, 3, H, Dh), 2, 0, 3, 1, 4)
        q, k, v = qkv[0], qkv[1], qkv[2]
        scores = jnp.einsum("bhqd,bhkd->bhqk", q, k) * (Dh ** -0.5)
        idx = jnp.arange(S)
        mask = (idx[:, None] - idx[None, :] >= 0) & (idx[:, None] - idx[None, :] < W)
        scores = jnp.where(mask[None, None], scores, -1e9)
        p = _softmax(scores, axis=-1)
        o = jnp.einsum("bhqk,bhkd->bhqd", p, v)
        return (lambda x, *d: x.transpose(*d))(o, 0, 2, 1, 3).reshape(B, S, D) @ wo

    def _B_ref(x, wqkv, wo):
        B, S, D = x.shape
        H = 32; Dh = D // H
        W, dil = 8, 2
        qkv = (lambda x, *d: x.transpose(*d))((x @ wqkv).reshape(B, S, 3, H, Dh), 2, 0, 3, 1, 4)
        q, k, v = qkv[0], qkv[1], qkv[2]
        scale = Dh ** -0.5
        pos = jnp.arange(S)
        off = jnp.arange(W) * dil
        idx = pos[:, None] - off[None, :]
        mask = idx >= 0
        idx_c = jnp.where(mask, idx, 0).reshape(-1)
        kg = k[:, :, idx_c, :].reshape(B, H, S, W, Dh)
        vg = v[:, :, idx_c, :].reshape(B, H, S, W, Dh)
        logits = jnp.einsum("bhsd,bhswd->bhsw", q, kg) * scale
        logits = jnp.where(mask[None, None, :, :], logits, -1e9)
        attn = _softmax(logits, axis=-1)
        o = jnp.einsum("bhsw,bhswd->bhsd", attn, vg)
        return (lambda x, *d: x.transpose(*d))(o, 0, 2, 1, 3).reshape(B, S, D) @ wo

    x = A_x
    x = x + _A_ref(_layernorm(x, axis=-1), A_wqkv, A_wo)
    x = x + _B_ref(_layernorm(x, axis=-1), B_wqkv, B_wo)
    x = x + _A_ref(_layernorm(x, axis=-1), A_wqkv, A_wo)
    x = x + _B_ref(_layernorm(x, axis=-1), B_wqkv, B_wo)
    return x
```

```python
import functools
import numpy as np
import jax
import jax.numpy as jnp
from jax import lax
from jax.experimental import pallas as pl
from jax.experimental.pallas import tpu as pltpu

S, D, H, DH = 2048, 1024, 32, 32
G = 8
TM = 256
NB = S // TM
QSCALE = float(DH ** -0.5 * np.log2(np.e))
NEG = -1e30
bf = jnp.bfloat16
i32 = jnp.int32
f32 = jnp.float32

def _pack_mask():
    ii = np.arange(64)[:, None]; cc = np.arange(128)[None, :]
    m = (np.where(cc >= 2*ii, 0xFFFF, 0) | np.where(cc >= 2*ii+1, 0xFFFF0000, 0)).astype(np.uint32)
    return m.view(np.int32)

def make(NC=256, only=None, lnsplit=2, scopes=False):
  NCH = 3*D // NC
  NCO = D // NC
  def kernel(x_hbm, wqkvA_hbm, woA_hbm, wqkvB_hbm, woB_hbm, mask_ref, out_hbm,
             x_s, h0, h1, q0_s, q1_s, k0_s, k1_s, v0_s, v1_s, o0_s, o1_s,
             wqkv_s, wo_s, xio_s, s0_s, s1_s, m0_s, m1_s, sems, osems):
    hS, qS, kS, vS, oS = (h0, h1), (q0_s, q1_s), (k0_s, k1_s), (v0_s, v1_s), (o0_s, o1_s)
    sS, mS = (s0_s, s1_s), (m0_s, m1_s)
    def xcopy(i):
        r = pl.ds(pl.multiple_of(i*TM, TM), TM)
        return pltpu.make_async_copy(x_hbm.at[0, r, :], xio_s.at[r, :], sems.at[i])
    def ocopy(i):
        r = pl.ds(pl.multiple_of(i*TM, TM), TM)
        return pltpu.make_async_copy(xio_s.at[r, :], out_hbm.at[0, r, :], osems.at[i])
    cwa = [pltpu.make_async_copy(wqkvA_hbm.at[:, pl.ds(c*512, 512)], wqkv_s.at[0, :, pl.ds(c*512, 512)], sems.at[NB+c]) for c in range(6)]
    cw = [pltpu.make_async_copy(woA_hbm, wo_s.at[0], sems.at[NB+6]),
          pltpu.make_async_copy(wqkvB_hbm, wqkv_s.at[1], sems.at[NB+7]),
          pltpu.make_async_copy(woB_hbm, wo_s.at[1], sems.at[NB+8])]
    xcopy(0).start()
    for c in cwa: c.start()
    xcopy(1).start()

    lane64 = lax.broadcasted_iota(i32, (64, 128), 1)
    rr = lax.broadcasted_iota(i32, (128, 128), 0)
    cc = lax.broadcasted_iota(i32, (128, 128), 1)

    def rows(i, part=0, n=TM):
        return pl.ds(pl.multiple_of(i*TM + part*n, n), n)

    def convert_in(i):
        xcopy(i).wait()
        x_s[rows(i), :] = xio_s[rows(i), :].astype(f32)

    def ln(i, p, part):
        n = TM // lnsplit
        xb = x_s[rows(i, part, n), :]
        m = jnp.mean(xb, axis=-1, keepdims=True)
        xc = xb - m
        v = jnp.mean(xc * xc, axis=-1, keepdims=True)
        hS[p][part*(n//2):(part+1)*(n//2), :] = pltpu.bitcast((xc * lax.rsqrt(v + 1e-5)).astype(bf), i32)

    def qkv_chunk(w, p, c):
        hb = pltpu.bitcast(hS[p][...], bf)
        acc = jnp.dot(hb, wqkv_s[w, :, c*NC:(c+1)*NC], preferred_element_type=f32)
        for j in range(NC // 128):
            col = c*NC + j*128
            kind, g = col // D, (col % D) // 128
            a = acc[:, j*128:(j+1)*128]
            if kind == 0:
                qS[p][g] = pltpu.bitcast((a * QSCALE).astype(bf), i32)
            elif kind == 1:
                kS[p][g, 128:256, :] = pltpu.bitcast(a.astype(bf), i32)
            else:
                vS[p][g, :, 256:512] = pltpu.bitcast(a.astype(bf).T, i32)

    def carry_kv(p, isA, g):
        if isA:
            kS[1-p][g, 0:128, :] = kS[p][g, 128:256, :]
            vS[1-p][g, :, 0:256] = vS[p][g, :, 256:512]
        else:
            kS[1-p][g, 120:128, :] = kS[p][g, 248:256, :]
            vS[1-p][g, :, 128:256] = vS[p][g, :, 384:512]

    def out_chunk(w, p, i, c):
        ob = pltpu.bitcast(oS[p][...], bf)
        y = x_s[rows(i), c*NC:(c+1)*NC] + jnp.dot(ob, wo_s[w, :, c*NC:(c+1)*NC], preferred_element_type=f32)
        x_s[rows(i), c*NC:(c+1)*NC] = y
        xio_s[rows(i), c*NC:(c+1)*NC] = y.astype(bf)

    def qmask(p, g, sub):
        qblk = qS[p][g, sub*64:(sub+1)*64, :]
        qm = jnp.concatenate([jnp.where(lane64//32 == h, qblk, 0) for h in range(4)], axis=0)
        return pltpu.bitcast(qm, bf)

    def qk(kk, qm):
        return lax.dot_general(kk, qm, (((1,), (1,)), ((), ())), preferred_element_type=f32)

    def store_o(outs, p, g, sub):
        ot = jnp.concatenate(outs, axis=0)
        oS[p][sub*64:(sub+1)*64, g*128:(g+1)*128] = pltpu.bitcast(ot.astype(bf).T, i32)

    def a_stage1(p, i, sub, g, slot, case):
        qm = qmask(p, g, sub)
        b = 128 + sub*64
        k0 = kS[p][g, b:b+64, :]
        tri = cc >= rr
        if case == 2:
            k2 = kS[p][g, b-128:b-64, :]; k1 = kS[p][g, b-64:b, :]
            parts = []
            for j in range(8):
                parts += [k2[j*8:(j+1)*8], k0[j*8:(j+1)*8]]
            st = qk(pltpu.bitcast(jnp.concatenate(parts + [k1], axis=0), bf), qm)
        elif case == 1:
            k1 = kS[p][g, b-64:b, :]
            st = qk(pltpu.bitcast(jnp.concatenate([k0, k1], axis=0), bf), qm)
        else:
            st = qk(pltpu.bitcast(k0, bf), qm)
        for h in range(4):
            sh = st[:, h*128:(h+1)*128]
            if case == 2:
                s2 = jnp.concatenate([sh[j*32:j*32+16] for j in range(8)], axis=0)
                s0 = jnp.concatenate([sh[j*32+16:j*32+32] for j in range(8)], axis=0)
                sc = jnp.where(tri, s0, s2)
                s1 = sh[256:384]
            else:
                sc = jnp.where(tri, sh[0:128], NEG)
                s1 = sh[128:256] if case == 1 else None
            sS[slot][h, 0:128] = sc
            if s1 is not None:
                sS[slot][h, 128:256] = s1
                sc = jnp.maximum(sc, s1)
            mS[slot][h] = jnp.max(sc, axis=0, keepdims=True)

    def a_stage2(p, i, sub, g, slot, case):
        n = 128 if case == 0 else 256
        outs = []
        for h in range(4):
            pr = jnp.exp2(sS[slot][h, 0:n] - mS[slot][h])
            l = jnp.sum(pr, axis=0, keepdims=True)
            pb = pltpu.bitcast(pr.astype(bf), i32)
            if case == 2:
                pc = pb[0:64]
                pcur = pc & mask_ref[...]
                pf = jnp.concatenate([pc ^ pcur, pb[64:128], pcur], axis=0)
            elif case == 1:
                pf = jnp.concatenate([pb[64:128], pb[0:64]], axis=0)
            else:
                pf = pb
            nk = 128*(case+1)
            e = 256 + (sub+1)*128
            vt = pltpu.bitcast(vS[p][g, h*16:(h+1)*16, e-nk:e], bf)
            ot = jnp.dot(vt, pltpu.bitcast(pf, bf), preferred_element_type=f32)
            outs.append(ot * (1.0 / l))
        store_o(outs, p, g, sub)

    rb = lax.broadcasted_iota(i32, (144, 128), 0)
    cb = lax.broadcasted_iota(i32, (144, 128), 1)
    def b_stage1(p, i, sub, g, slot, case):
        qm = qmask(p, g, sub)
        b = 128 + sub*64
        st = qk(pltpu.bitcast(kS[p][g, b-8:b+64, :], bf), qm)
        d = cb + 16 - rb
        ok = (d >= 0) & (d <= 14) & ((d & 1) == 0)
        ok16 = ok[0:16]
        if sub == 0:
            ok16 = ok16 & (jnp.zeros((16, 128), i32) + i > 0)
        for h in range(4):
            sh = st[:, h*128:(h+1)*128]
            sa = jnp.where(ok16, sh[0:16], NEG)
            sb = jnp.where(ok[16:144], sh[16:144], NEG)
            sS[slot][h, 0:16] = sa
            sS[slot][h, 16:144] = sb
            mS[slot][h] = jnp.maximum(jnp.max(sa, axis=0, keepdims=True), jnp.max(sb, axis=0, keepdims=True))

    def b_stage2(p, i, sub, g, slot, case):
        outs = []
        for h in range(4):
            pr = jnp.exp2(sS[slot][h, 0:144] - mS[slot][h])
            l = jnp.sum(pr, axis=0, keepdims=True)
            pf = jnp.concatenate([jnp.zeros((112, 128), bf), pr.astype(bf)], axis=0)
            e = 256 + (sub+1)*128
            vt = pltpu.bitcast(vS[p][g, h*16:(h+1)*16, e-256:e], bf)
            ot = jnp.dot(vt, pf, preferred_element_type=f32)
            outs.append(ot * (1.0 / l))
        store_o(outs, p, g, sub)

    def step(t, p, isA, first=False, do_qkv=True, do_ln=True, do_out=True):
        i = t % NB
        s1, s2 = (a_stage1, a_stage2) if isA else (b_stage1, b_stage2)
        units = [(sub, g, (sub if first else 2) if isA else 0) for sub in range(2) for g in range(G)]
        work = []
        if do_out:
            for c in range(NCO):
                work.append(functools.partial(out_chunk, ((t-1)//NB) % 2, 1-p, (t-1) % NB, c))
        if do_qkv:
            late = [functools.partial(ln, (t+2) % NB, p, part) for part in range(lnsplit)] if do_ln else []
            for c in range(NCH):
                work.append(functools.partial(qkv_chunk, ((t+1)//NB) % 2, 1-p, c))
                if c < len(late): work.append(late[c])
        nu = len(units)
        wi = 0
        s1(p, i, units[0][0], units[0][1], 0, units[0][2])
        for u in range(nu):
            if u + 1 < nu:
                s1(p, i, units[u+1][0], units[u+1][1], (u+1) % 2, units[u+1][2])
            tgt = (len(work) * (u + 1) + nu - 1) // nu
            while wi < min(tgt, len(work)):
                work[wi](); wi += 1
            if do_qkv and u < G:
                carry_kv(p, isA, u)
            s2(p, i, units[u][0], units[u][1], u % 2, units[u][2])

    def pair(P, isA, first=False, last=False):
        t = 2*P
        if isA:
            if P < 3:
                convert_in(t + 2); convert_in(t + 3)
        else:
            @pl.when(P >= 13)
            def _():
                ocopy(t - 2 - 24).start()
                @pl.when(P >= 14)
                def _():
                    ocopy(t - 3 - 24).start()
        if first:
            step(t, 0, isA, first=True, do_out=P > 0)
            if P == 0:
                cw[0].wait()
        else:
            step(t, 0, isA, do_ln=not last)
        step(t + 1, 1, isA, do_qkv=not last)

    vS[0][:, :, 128:256] = jnp.zeros((G, 64, 128), i32)
    kS[0][:, 120:128, :] = jnp.zeros((G, 8, 128), i32)
    convert_in(0)
    for part in range(lnsplit): ln(0, 0, part)
    for c in range(6):
        cwa[c].wait()
        if c == 0:
            for i in range(2, NB): xcopy(i).start()
            cw[0].start()
        for cc_ in range(512 // NC):
            qkv_chunk(0, 0, c*(512//NC) + cc_)
    cw[1].start(); cw[2].start()
    convert_in(1)
    for part in range(lnsplit): ln(1, 1, part)

    def macro(m, carry):
        pair(8*m, True, first=True)
        def bodyA(P, c):
            if P == 3:
                cw[1].wait(); cw[2].wait()
            pair(P, True)
            return c
        for j in range(1, 4): bodyA(8*m + j, 0)
        def bodyB(P, c):
            pair(P, False)
            return c
        lax.fori_loop(8*m + 4, 8*m + 8 - m, bodyB, 0)
        return carry
    macro(0, 0); macro(1, 0)
    pair(15, False, last=True)
    ocopy(5).start(); ocopy(6).start()
    for c in range(NCO):
        out_chunk(1, 1, NB-1, c)
    ocopy(7).start()
    for i in range(NB):
        ocopy(i).wait()

  MASK = _pack_mask()
  def fn(A_x, A_wqkv, A_wo, B_x, B_wqkv, B_wo):
    anyspec = pl.BlockSpec(memory_space=pl.ANY)
    vm = pl.BlockSpec(memory_space=pltpu.VMEM)
    V = pltpu.VMEM
    return pl.pallas_call(
        kernel,
        out_shape=jax.ShapeDtypeStruct((1, S, D), bf),
        in_specs=[anyspec]*5 + [vm],
        out_specs=anyspec,
        scratch_shapes=[
            V((S, D), f32), V((TM//2, D), i32), V((TM//2, D), i32),
            V((G, 128, 128), i32), V((G, 128, 128), i32),
            V((G, 256, 128), i32), V((G, 256, 128), i32),
            V((G, 64, 512), i32), V((G, 64, 512), i32),
            V((TM//2, D), i32), V((TM//2, D), i32),
            V((2, D, 3*D), bf), V((2, D, D), bf),
            V((S, D), bf),
            V((4, 256, 128), f32), V((4, 256, 128), f32), V((4, 1, 128), f32), V((4, 1, 128), f32),
            pltpu.SemaphoreType.DMA((NB + 9,)), pltpu.SemaphoreType.DMA((NB,)),
        ],
        compiler_params=pltpu.CompilerParams(vmem_limit_bytes=100*1024*1024),
        name="fused",
    )(A_x, A_wqkv, A_wo, B_wqkv, B_wo, jnp.asarray(MASK))
  return fn


_fn = make()

@jax.jit
def pallas_interleave_layers__sliding_block__sliding_local_dilated__prompt_kernel(
    A_x: jax.Array, A_wqkv: jax.Array, A_wo: jax.Array,
    B_x: jax.Array, B_wqkv: jax.Array, B_wo: jax.Array,
):
    return _fn(A_x, A_wqkv, A_wo, B_x, B_wqkv, B_wo)
```
